```python
import jax
import jax.numpy as jnp

def _softmax(x, axis=-1):
    return jax.nn.softmax(x, axis=axis)
def _gelu(x):
    return jax.nn.gelu(x, approximate=True)
def _silu(x):
    return jax.nn.silu(x)
def _sigmoid(x):
    return jax.nn.sigmoid(x)
def _layernorm(x, axis=-1, eps=1e-5):
    m = jnp.mean(x, axis=axis, keepdims=True)
    v = jnp.var(x, axis=axis, keepdims=True)
    return (x - m) / jnp.sqrt(v + eps)
def _scatter_add(tgt, idx, src, axis=0):
    return tgt.at[idx].add(src)
def _segment_sum(src, seg, n):
    return jax.ops.segment_sum(src, seg, n)
class _Rng:
    def __init__(self, key):
        self._k = key
    def _next(self):
        self._k, sub = jax.random.split(self._k)
        return sub
    def normal(self, shape):
        return jax.random.normal(self._next(), shape, dtype=jnp.bfloat16)
    def randint(self, lo, hi, shape):
        return jax.random.randint(self._next(), shape, lo, hi, dtype=jnp.int32)
    def uniform(self, shape, lo=0.0, hi=1.0):
        return jax.random.uniform(self._next(), shape, jnp.bfloat16, lo, hi)
    def permutation(self, n):
        return jax.random.permutation(self._next(), n)


kernel_name = 'sequential_preLN__spectral_gfnet__swiglu_ffn__prompt'

def _fwd_setup_inputs():
    _rng = _Rng(jax.random.key(int.from_bytes(__import__("os").urandom(4), "little")))
    _w = (lambda a: (lambda t: t.astype(jnp.bfloat16) if jnp.issubdtype(t.dtype, jnp.floating) else t)(jnp.asarray(a)))
    def _A_setup():
        B, S, D = 1, 2048, 576
        Df = D // 2 + 1
        return {
            "x": _w((lambda *s: _rng.normal(s) * 0.05)(B, S, D)),
            "w_r": _w((lambda *s: _rng.normal(s) * 0.05)(S, Df) * 0.02),
            "w_i": _w((lambda *s: _rng.normal(s) * 0.05)(S, Df) * 0.02),
        }
    _A_in = _A_setup()

    def _B_setup():
        B, S, D, F = 1, 2048, 576, 4608
        return {
            "x": _w((lambda *s: _rng.normal(s) * 0.05)(B, S, D)),
            "w_gate": _w((lambda *s: _rng.normal(s) * 0.05)(D, F)),
            "w_up": _w((lambda *s: _rng.normal(s) * 0.05)(D, F)),
            "w_down": _w((lambda *s: _rng.normal(s) * 0.05)(F, D)),
        }
    _B_in = _B_setup()

    return {
        "A_x": _A_in["x"],
        "A_w_r": _A_in["w_r"],
        "A_w_i": _A_in["w_i"],
        "B_x": _B_in["x"],
        "B_w_gate": _B_in["w_gate"],
        "B_w_up": _B_in["w_up"],
        "B_w_down": _B_in["w_down"],
    }

def _fwd_reference(A_x, A_w_r, A_w_i, B_x, B_w_gate, B_w_up, B_w_down):
    def _A_ref(x, w_r, w_i):
        B, S, D = x.shape
        X = (lambda x, axes=(-2,-1): jnp.fft.rfft2(x.astype(jnp.float32), axes=axes))(x, axes=(-2, -1))
        W = w_r + 1j * w_i
        X = X * W
        y = (lambda x, s, axes=(-2,-1): jnp.fft.irfft2(x, s=s, axes=axes).astype(jnp.bfloat16))(X, (S, D), axes=(-2, -1))
        return y

    def _B_ref(x, w_gate, w_up, w_down):
        g = _silu(x @ w_gate)
        u = x @ w_up
        return (g * u) @ w_down

    x = A_x
    h = x + _A_ref(_layernorm(x, axis=-1), A_w_r, A_w_i)
    h2 = h + _B_ref(_layernorm(h, axis=-1), B_w_gate, B_w_up, B_w_down)
    return h2


def setup_inputs():
    _inp = _fwd_setup_inputs()
    _gk = jax.random.fold_in(jax.random.key(int.from_bytes(__import__("os").urandom(4), "little")), 2**31 - 1)
    _shapes = [[1, 2048, 576]]
    _dtypes = ['bfloat16']
    _gks = jax.random.split(_gk, len(_shapes))
    _gs = [jax.random.normal(k, s, dtype=jnp.dtype(d)) * 0.05 for k, s, d in zip(_gks, _shapes, _dtypes)]
    _inp["grad_out"] = _gs[0]
    return _inp

def reference(A_x, A_w_r, A_w_i, B_w_gate, B_w_up, B_w_down, B_x, grad_out):
    _const = dict(B_x=B_x)
    def _f(*_d):
        return _fwd_reference(**{'A_x': _d[0], 'A_w_r': _d[1], 'A_w_i': _d[2], 'B_w_gate': _d[3], 'B_w_up': _d[4], 'B_w_down': _d[5], **_const})
    _out, _vjp = jax.vjp(_f, A_x, A_w_r, A_w_i, B_w_gate, B_w_up, B_w_down)
    _grads = _vjp(grad_out)
    _out0 = jnp.asarray(_out)
    return (_out0, *[jnp.asarray(_g) for _g in _grads])
```

```python
import math

import numpy as np
import jax
import jax.numpy as jnp
from jax import lax
import jax.experimental.pallas as pl
import jax.experimental.pallas.tpu as pltpu

S, D, DF, F = 2048, 576, 289, 4608
LP = 304
R2 = 2 * LP
DH = D // 2
NE = 145
EP = 160
NO = 144
NB = 16
TF = 512
NT_F = F // TF
SC = 1024
CH = 256
KU = 4
DWU = True
CU = 1
EPS = 1e-5
BF = jnp.bfloat16
F32 = jnp.float32
U32 = jnp.uint32

_PROF = False


def _loop(name, n, body, unroll=1):
    if _PROF:
        with jax.named_scope(name):
            lax.fori_loop(0, n, body, 0, unroll=unroll)
    else:
        lax.fori_loop(0, n, body, 0, unroll=unroll)


_NN = (((1,), (0,)), ((), ()))
_NT = (((1,), (1,)), ((), ()))
_TN = (((0,), (0,)), ((), ()))


def _mm(a, b, dn):
    return lax.dot_general(a, b, dn, preferred_element_type=F32)


def _bfly4(ar, ai, sg):
    t0r, t0i = ar[0] + ar[2], ai[0] + ai[2]
    t1r, t1i = ar[0] - ar[2], ai[0] - ai[2]
    t2r, t2i = ar[1] + ar[3], ai[1] + ai[3]
    t3r, t3i = ar[1] - ar[3], ai[1] - ai[3]
    x0r, x0i = t0r + t2r, t0i + t2i
    x2r, x2i = t0r - t2r, t0i - t2i
    if sg > 0:
        x1r, x1i = t1r - t3i, t1i + t3r
        x3r, x3i = t1r + t3i, t1i - t3r
    else:
        x1r, x1i = t1r + t3i, t1i - t3r
        x3r, x3i = t1r - t3i, t1i + t3r
    return [x0r, x1r, x2r, x3r], [x0i, x1i, x2i, x3i]


def _tw16(r, m, j, sg):
    j = j % 16
    if j == 0:
        return r, m
    if j == 4:
        return (-m, r) if sg > 0 else (m, -r)
    c = np.float32(math.cos(2 * math.pi * j / 16))
    d = np.float32(sg * math.sin(2 * math.pi * j / 16))
    if j in (2, 6):
        if c == d:
            return (r - m) * c, (r + m) * c
        else:
            return (r + m) * c, (m - r) * c
    return r * c - m * d, r * d + m * c


def _fft16(xr, xi, sg):
    tr = [None] * 4
    ti = [None] * 4
    for nb in range(4):
        br, bi = _bfly4([xr[4 * na + nb] for na in range(4)],
                        [xi[4 * na + nb] for na in range(4)], sg)
        for ka in range(4):
            br[ka], bi[ka] = _tw16(br[ka], bi[ka], nb * ka, sg)
        tr[nb], ti[nb] = br, bi
    yr = [None] * 16
    yi = [None] * 16
    for ka in range(4):
        br, bi = _bfly4([tr[nb][ka] for nb in range(4)],
                        [ti[nb][ka] for nb in range(4)], sg)
        for kb in range(4):
            yr[ka + 4 * kb] = br[kb]
            yi[ka + 4 * kb] = bi[kb]
    return yr, yi


def _radix16_stage(buf, sg):
    def body(t, c):
        r = pl.multiple_of(t * 8, 8)
        ri = pl.multiple_of(t * 8 + LP, 8)
        xr = [buf[pl.ds(r, 8), n * 128:(n + 1) * 128] for n in range(NB)]
        xi = [buf[pl.ds(ri, 8), n * 128:(n + 1) * 128] for n in range(NB)]
        yr, yi = _fft16(xr, xi, sg)
        for k in range(NB):
            buf[pl.ds(r, 8), k * 128:(k + 1) * 128] = yr[k]
            buf[pl.ds(ri, 8), k * 128:(k + 1) * 128] = yi[k]
        return c
    _loop('r16', LP // 8, body)


def _ln_stats(v):
    mu = jnp.mean(v, axis=0, keepdims=True)
    vc = v - mu
    var = jnp.mean(vc * vc, axis=0, keepdims=True)
    rstd = lax.rsqrt(var + EPS)
    return vc * rstd, rstd


def _ln_bwd(dn, vhat, rstd):
    m1 = jnp.mean(dn, axis=0, keepdims=True)
    m2 = jnp.mean(dn * vhat, axis=0, keepdims=True)
    return rstd * (dn - m1 - vhat * m2)


def _pack2(a_bf, b_bf):
    ah = lax.bitcast_convert_type(a_bf.astype(F32), U32)
    bh = lax.bitcast_convert_type(b_bf.astype(F32), U32)
    return ah | (bh >> 16)


def _unpack2(p):
    a = lax.bitcast_convert_type(p & np.uint32(0xFFFF0000), F32)
    b = lax.bitcast_convert_type(p << 16, F32)
    return a, b


def _lane(i, n):
    return pl.ds(pl.multiple_of(i * n, n), n)


def _kernel(x_hbm, wr_hbm, wi_hbm, wg_hbm, wu_hbm, wd_hbm, go_hbm,
            out_hbm, dx_hbm, dwr_hbm, dwi_hbm, dwg_hbm, dwu_hbm, dwd_hbm,
            xv, lhs, wrv, wiv, hT, n1T, rs, outT, dn2T, Xs, WT, bufA, bufB, CE, CO, CEt, COt, Tf,
            wtmp, stg, hb, wbuf, dwbuf, ov, dxv,
            sem_in, sem_w, sem_dw, sem_out, sem_fin):

    n2T = lhs.at[0]
    gov = lhs.at[1]

    def w_copy(t, slot, which):
        src = (wg_hbm, wu_hbm, wd_hbm)[which]
        return pltpu.make_async_copy(src.at[:, _lane(t, TF)], wbuf.at[slot, which],
                                     sem_w.at[slot, which])

    def dw_copy(t, slot, which):
        dst = (dwg_hbm, dwu_hbm, dwd_hbm)[which]
        return pltpu.make_async_copy(dwbuf.at[slot, which], dst.at[:, _lane(t, TF)],
                                     sem_dw.at[slot, which])

    def in_copies(c):
        cols = _lane(c, CH)
        return (pltpu.make_async_copy(x_hbm.at[:, cols], xv.at[:, cols], sem_in.at[c, 0]),
                pltpu.make_async_copy(wr_hbm.at[:, cols], wrv.at[:, cols], sem_in.at[c, 1]),
                pltpu.make_async_copy(wi_hbm.at[:, cols], wiv.at[:, cols], sem_in.at[c, 2]))

    for c in range(S // CH):
        for cp in in_copies(c):
            cp.start()
    cp_go = pltpu.make_async_copy(go_hbm, gov, sem_out.at[1])

    def row_scale(nrows, base):
        lrow = lax.broadcasted_iota(jnp.int32, (nrows, 128), 0) + base
        return jnp.where((lrow == 0) | (lrow == NE - 1), np.float32(1.0 / (S * D)),
                         np.float32(2.0 / (S * D)))

    def dfwd(v, cols):
        e = (v[:DH] + v[DH:]).astype(BF)
        o = (v[:DH] - v[DH:]).astype(BF)
        pe = _mm(CE[...], e, _NN)
        po = _mm(CO[...], o, _NN)
        bufA[0:EP, cols] = pe[:EP]
        bufA[EP:LP, cols] = po[:NO]
        bufA[LP:LP + EP, cols] = pe[EP:]
        bufA[LP + EP:R2, cols] = po[NO:]

    def dinv(cols):
        ze = jnp.concatenate([bufB[0:EP, cols], bufB[LP:LP + EP, cols]], axis=0).astype(BF)
        zo = jnp.concatenate([bufB[EP:LP, cols], bufB[LP + EP:R2, cols]], axis=0).astype(BF)
        ee = _mm(CEt[...], ze, _NN)
        oo = _mm(COt[...], zo, _NN)
        return jnp.concatenate([ee + oo, ee - oo], axis=0)

    def spectral(mid):
        _radix16_stage(bufA, -1)

        def blk(k1):
            cols = _lane(k1, 128)
            a = jnp.concatenate([bufA[0:LP, cols], bufA[LP:R2, cols]], axis=1).astype(BF)
            q = _mm(a, Tf[k1], _NN)
            yr, yi = mid(k1, cols, q[:, 0:128], q[:, 128:256])
            y = jnp.concatenate([yr, yi], axis=1).astype(BF)
            p = _mm(y, Tf[k1], _NT)
            bufB[0:LP, cols] = p[:, 0:128]
            bufB[LP:R2, cols] = p[:, 128:256]

        def blk2(k2, c):
            blk(2 * k2)
            blk(2 * k2 + 1)
            return c
        _loop('kblk', NB // 2, blk2, unroll=KU // 2)
        _radix16_stage(bufB, +1)

    row = lax.broadcasted_iota(jnp.int32, (16, DH), 0)
    col = lax.broadcasted_iota(jnp.int32, (16, DH), 1)

    def _ang(m):
        m = m.astype(F32)
        m = m - jnp.floor(m * np.float32(1.0 / D)) * np.float32(D)
        m = jnp.where(m < 0, m + D, m)
        m = jnp.where(m >= D, m - D, m)
        return m * np.float32(2 * math.pi / D)
    ae = _ang(2 * row * col)
    ao = _ang((2 * row + 1) * col)
    av = _ang(32 * col)
    vr, vi = jnp.cos(av), -jnp.sin(av)

    def cs_body(t, carry):
        er, ei, orr, oi = carry
        valid = (row + t * 16) < NE
        CE[pl.ds(pl.multiple_of(t * 16, 16), 16), :] = jnp.where(valid, er, 0.0).astype(BF)
        CE[pl.ds(pl.multiple_of(t * 16 + EP, 16), 16), :] = jnp.where(valid, ei, 0.0).astype(BF)

        @pl.when(t < NO // 16)
        def _():
            CO[pl.ds(pl.multiple_of(t * 16, 16), 16), :] = orr.astype(BF)
            CO[pl.ds(pl.multiple_of(t * 16 + NO, 16), 16), :] = oi.astype(BF)
        return (er * vr - ei * vi, er * vi + ei * vr, orr * vr - oi * vi, orr * vi + oi * vr)
    lax.fori_loop(0, EP // 16, cs_body, (jnp.cos(ae), -jnp.sin(ae), jnp.cos(ao), -jnp.sin(ao)))

    CEt[...] = CE[...].T
    COt[...] = CO[...].T

    n2i = lax.broadcasted_iota(jnp.int32, (128, 128), 0)
    k2i = lax.broadcasted_iota(jnp.int32, (128, 128), 1)
    b0 = ((n2i * (NB * k2i)) & (S - 1)).astype(F32) * np.float32(2 * math.pi / S)
    bv = n2i.astype(F32) * np.float32(2 * math.pi / S)
    ur, ui = jnp.cos(bv), -jnp.sin(bv)

    def t_body(k1, carry):
        tr, ti = carry
        trb, tib = tr.astype(BF), ti.astype(BF)
        Tf[k1, 0:128, 0:128] = trb
        Tf[k1, 0:128, 128:256] = tib
        Tf[k1, 128:256, 0:128] = -tib
        Tf[k1, 128:256, 128:256] = trb
        return tr * ur - ti * ui, tr * ui + ti * ur
    lax.fori_loop(0, NB, t_body, (jnp.cos(b0), -jnp.sin(b0)))

    wtmp[pl.ds(288, 32), :] = jnp.zeros((32, 128), U32)

    def a1_body(c, carry):
        cols = _lane(c, CH)
        for cp in in_copies(c):
            cp.wait()
        n1, rstd1 = _ln_stats(xv[:, cols].astype(F32))
        n1T[:, cols] = n1.astype(BF)
        rs[0:1, cols] = rstd1
        dfwd(n1, cols)
        for bb in range(CH // 128):
            bc = _lane(c * (CH // 128) + bb, 128)
            wtmp[0:DF, :] = _pack2(wrv[:, bc], wiv[:, bc])
            t0 = wtmp[pl.ds(0, 128, stride=2), :]
            t1 = jnp.concatenate([wtmp[pl.ds(256, EP - 128, stride=2), :],
                                  wtmp[pl.ds(1, 256 - EP, stride=2), :]], axis=0)
            t2 = jnp.concatenate([wtmp[pl.ds(1 + 2 * (256 - EP), LP - 256, stride=2), :],
                                  jnp.zeros((384 - LP, 128), U32)], axis=0)
            stg[0, bc, :] = t0.T
            stg[1, bc, :] = t1.T
            stg[2, bc, :] = t2.T
        return carry
    _loop('a1', S // CH, a1_body, unroll=CU)
    cp_go.start()
    for which in range(3):
        w_copy(0, 0, which).start()

    def mid_a(k1, cols, xr, xi):
        for j in range(3):
            nr = 128 if j < 2 else LP - 256
            p = stg[j, pl.ds(k1, 128, stride=NB), :].T
            w_r, w_i = _unpack2(p[0:nr])
            scj = row_scale(nr, j * 128)
            WT[j * 128:j * 128 + nr, cols] = w_r * scj
            WT[LP + j * 128:LP + j * 128 + nr, cols] = w_i * scj
        sc = row_scale(LP, 0)
        Xs[0:LP, cols] = xr * sc
        Xs[LP:R2, cols] = xi * sc
        w_r = WT[0:LP, cols]
        w_i = WT[LP:R2, cols]
        return xr * w_r - xi * w_i, xr * w_i + xi * w_r

    spectral(mid_a)

    def a2_body(c, carry):
        cols = _lane(c, CH)
        y = dinv(cols)
        h = (xv[:, cols].astype(F32) + y.astype(BF).astype(F32)).astype(BF).astype(F32)
        hT[:, cols] = h
        n2, rstd2 = _ln_stats(h)
        n2T[:, cols] = n2.astype(BF)
        rs[8:9, cols] = rstd2
        outT[:, cols] = jnp.zeros((D, CH), F32)
        dn2T[:, cols] = jnp.zeros((D, CH), F32)
        return carry
    _loop('a2', S // CH, a2_body, unroll=CU)
    cp_go.wait()

    def tile(t, carry):
        slot = t % 2

        @pl.when(t + 1 < NT_F)
        def _():
            for which in range(3):
                w_copy(t + 1, 1 - slot, which).start()

        for which in range(3):
            w_copy(t, slot, which).wait()

        def chunk(c, carry2):
            cols = _lane(c, SC)
            n2c = n2T[:, cols]
            doc = gov[:, cols]
            wg = wbuf[slot, 0]
            wu = wbuf[slot, 1]
            wd = wbuf[slot, 2]
            g = _mm(wg, n2c, _TN)
            u = _mm(wu, n2c, _TN)
            da = _mm(wd, doc, _TN)
            sig = 1.0 / (1.0 + jnp.exp(-g))
            gs = g * sig
            a_b = (gs * u).astype(BF)
            du_b = (da * gs).astype(BF)
            dg_b = (da * u * (sig * (1.0 + g * (1.0 - sig)))).astype(BF)
            hb[2, :, cols] = a_b
            hb[1, :, cols] = du_b
            hb[0, :, cols] = dg_b
            outT[:, cols] += _mm(wd, a_b, _NN)
            dn2T[:, cols] += _mm(wg, dg_b, _NN) + _mm(wu, du_b, _NN)
            return carry2
        _loop('chunks', S // SC, chunk)

        @pl.when(t >= 2)
        def _():
            for which in range(3):
                dw_copy(t - 2, slot, which).wait()

        def dw_body(i, carry2):
            dwbuf[slot, i] = _mm(lhs[i // 2], hb[i], _NT).astype(BF)
            return carry2
        lax.fori_loop(0, 3, dw_body, 0, unroll=DWU)
        for which in range(3):
            dw_copy(t, slot, which).start()
        return carry
    _loop('ffn', NT_F, tile)

    def c1_body(c, carry):
        cols = _lane(c, CH)
        h = hT[:, cols]
        ov[:, cols] = (h + outT[:, cols].astype(BF).astype(F32)).astype(BF)
        dh = (gov[:, cols].astype(F32)
              + _ln_bwd(dn2T[:, cols], n2T[:, cols].astype(F32), rs[8:9, cols])).astype(BF)
        hT[:, cols] = dh.astype(F32)
        dfwd(dh.astype(F32), cols)
        return carry
    _loop('c1', S // CH, c1_body, unroll=CU)
    cp_out = pltpu.make_async_copy(ov, out_hbm, sem_out.at[0])
    cp_out.start()

    def mid_c(k1, cols, gr, gi):
        x_r = Xs[0:LP, cols]
        x_i = Xs[LP:R2, cols]
        dwr = gr * x_r + gi * x_i
        dwi = gi * x_r - gr * x_i
        pk = _pack2(dwr.astype(BF), dwi.astype(BF))
        stg[0, pl.ds(k1, 128, stride=NB), :] = pk[0:128].T
        stg[1, pl.ds(k1, 128, stride=NB), :] = pk[128:256].T
        stg[2, pl.ds(k1, 128, stride=NB), :] = jnp.concatenate(
            [pk[256:LP], jnp.zeros((384 - LP, 128), U32)], axis=0).T
        w_r = WT[0:LP, cols]
        w_i = WT[LP:R2, cols]
        return gr * w_r + gi * w_i, gi * w_r - gr * w_i

    spectral(mid_c)

    def fin_copies(c):
        cols = _lane(c, CH)
        return (pltpu.make_async_copy(dxv.at[:, cols], dx_hbm.at[:, cols], sem_fin.at[c, 0]),
                pltpu.make_async_copy(wrv.at[:, cols], dwr_hbm.at[:, cols], sem_fin.at[c, 1]),
                pltpu.make_async_copy(wiv.at[:, cols], dwi_hbm.at[:, cols], sem_fin.at[c, 2]))

    def c2_body(c, carry):
        cols = _lane(c, CH)
        dn1 = dinv(cols)
        dx = hT[:, cols] + _ln_bwd(dn1, n1T[:, cols].astype(F32), rs[0:1, cols])
        dxv[:, cols] = dx.astype(BF)
        for bb in range(CH // 128):
            bc = _lane(c * (CH // 128) + bb, 128)
            p = jnp.concatenate([stg[j, bc, :].T for j in range(3)], axis=0)
            wtmp[pl.ds(0, NE, stride=2), :] = p[0:NE]
            wtmp[pl.ds(1, NO, stride=2), :] = p[EP:LP]
            d_r, d_i = _unpack2(wtmp[0:DF, :])
            wrv[:, bc] = d_r.astype(BF)
            wiv[:, bc] = d_i.astype(BF)
        for cp in fin_copies(c):
            cp.start()
        return carry
    _loop('c2', S // CH, c2_body, unroll=CU)

    for t in (NT_F - 2, NT_F - 1):
        for which in range(3):
            dw_copy(t, t % 2, which).wait()
    cp_out.wait()
    for c in range(S // CH):
        for cp in fin_copies(c):
            cp.wait()


@jax.jit
def pallas_sequential_preLN__spectral_gfnet__swiglu_ffn__prompt_kernel(
    A_x: jax.Array,
    A_w_r: jax.Array,
    A_w_i: jax.Array,
    B_x: jax.Array,
    B_w_gate: jax.Array,
    B_w_up: jax.Array,
    B_w_down: jax.Array,
    grad_out: jax.Array,
):
    x = A_x.reshape(S, D).T
    go = grad_out.reshape(S, D).T
    anyspec = pl.BlockSpec(memory_space=pl.ANY)
    out_shape = [
        jax.ShapeDtypeStruct((D, S), BF), jax.ShapeDtypeStruct((D, S), BF),
        jax.ShapeDtypeStruct((DF, S), BF), jax.ShapeDtypeStruct((DF, S), BF),
        jax.ShapeDtypeStruct((D, F), BF), jax.ShapeDtypeStruct((D, F), BF),
        jax.ShapeDtypeStruct((D, F), BF),
    ]
    scratch = [
        pltpu.VMEM((D, S), BF),
        pltpu.VMEM((2, D, S), BF),
        pltpu.VMEM((DF, S), BF),
        pltpu.VMEM((DF, S), BF),
        pltpu.VMEM((D, S), F32),
        pltpu.VMEM((D, S), BF),
        pltpu.VMEM((16, S), F32),
        pltpu.VMEM((D, S), F32),
        pltpu.VMEM((D, S), F32),
        pltpu.VMEM((R2, S), F32),
        pltpu.VMEM((R2, S), F32),
        pltpu.VMEM((R2, S), F32),
        pltpu.VMEM((R2, S), F32),
        pltpu.VMEM((2 * EP, DH), BF),
        pltpu.VMEM((2 * NO, DH), BF),
        pltpu.VMEM((DH, 2 * EP), BF),
        pltpu.VMEM((DH, 2 * NO), BF),
        pltpu.VMEM((NB, 256, 256), BF),
        pltpu.VMEM((320, 128), U32),
        pltpu.VMEM((3, S, 128), U32),
        pltpu.VMEM((3, TF, S), BF),
        pltpu.VMEM((2, 3, D, TF), BF),
        pltpu.VMEM((2, 3, D, TF), BF),
        pltpu.VMEM((D, S), BF),
        pltpu.VMEM((D, S), BF),
        pltpu.SemaphoreType.DMA((S // CH, 3)),
        pltpu.SemaphoreType.DMA((2, 3)),
        pltpu.SemaphoreType.DMA((2, 3)),
        pltpu.SemaphoreType.DMA((2,)),
        pltpu.SemaphoreType.DMA((S // CH, 3)),
    ]
    out, dx, dwr, dwi, dwg, dwu, dwd = pl.pallas_call(
        _kernel,
        in_specs=[anyspec] * 7,
        out_specs=[anyspec] * 7,
        out_shape=out_shape,
        scratch_shapes=scratch,
        compiler_params=pltpu.CompilerParams(vmem_limit_bytes=110 * 1024 * 1024),
    )(x, A_w_r.T, A_w_i.T, B_w_gate, B_w_up, B_w_down.T, go)
    return (out.T.reshape(1, S, D), dx.T.reshape(1, S, D), dwr.T, dwi.T, dwg, dwu, dwd.T)
```
